```python
import os as _os
_os.environ.setdefault("JAX_PLATFORMS", "cpu")
import jax
import jax.numpy as jnp

def _softmax(x, axis=-1):
    return jax.nn.softmax(x, axis=axis)
def _gelu(x):
    return jax.nn.gelu(x, approximate=True)
def _silu(x):
    return jax.nn.silu(x)
def _sigmoid(x):
    return jax.nn.sigmoid(x)
def _layernorm(x, axis=-1, eps=1e-5):
    m = jnp.mean(x, axis=axis, keepdims=True)
    v = jnp.var(x, axis=axis, keepdims=True)
    return (x - m) / jnp.sqrt(v + eps)
def _scatter_add(tgt, idx, src, axis=0):
    return tgt.at[idx].add(src)
def _segment_sum(src, seg, n):
    return jax.ops.segment_sum(src, seg, n)
class _Rng:
    def __init__(self, key):
        self._k = key
    def _next(self):
        self._k, sub = jax.random.split(self._k)
        return sub
    def normal(self, shape):
        return jax.random.normal(self._next(), shape, dtype=jnp.bfloat16)
    def randint(self, lo, hi, shape):
        return jax.random.randint(self._next(), shape, lo, hi, dtype=jnp.int32)
    def uniform(self, shape, lo=0.0, hi=1.0):
        return jax.random.uniform(self._next(), shape, jnp.bfloat16, lo, hi)
    def permutation(self, n):
        return jax.random.permutation(self._next(), n)


kernel_name = 'standalone__mha_block_cached__near_ridge'

def setup_inputs():
    _rng = _Rng(jax.random.key(int.from_bytes(__import__("os").urandom(4), "little")))
    _w = (lambda a: (lambda t: t.astype(jnp.bfloat16) if jnp.issubdtype(t.dtype, jnp.floating) else t)(jnp.asarray(a)))
    B, Sq, D = 8, 144, 448
    H, Sk, Dh = 16, 2048, 256
    return {
        "x": _w((lambda *s: _rng.normal(s) * 0.8)(B, Sq, D)),
        "k_cache": _w((lambda *s: _rng.normal(s) * 0.8)(B, H, Sk, Dh)),
        "v_cache": _w((lambda *s: _rng.normal(s) * 0.05)(B, H, Sk, Dh)),
        "wq": _w((lambda *s: _rng.normal(s) * 0.8)(D, H * Dh) * (D ** -0.5)),
        "wo": _w((lambda *s: _rng.normal(s) * 0.05)(H * Dh, D) * ((H * Dh) ** -0.5)),
    }

def reference(x, k_cache, v_cache, wq, wo):
    B, Sq, D = x.shape
    H, Dh = 16, 256
    q = (lambda x, *d: x.transpose(*d))((x @ wq).reshape(B, Sq, H, Dh), 0, 2, 1, 3)
    scores = jnp.einsum("bhqd,bhkd->bhqk", q, k_cache) * (Dh ** -0.5)
    p = _softmax(scores, axis=-1)
    o = jnp.einsum("bhqk,bhkd->bhqd", p, v_cache)
    return (lambda x, *d: x.transpose(*d))(o, 0, 2, 1, 3).reshape(B, Sq, H * Dh) @ wo
```

```python
import jax
import jax.numpy as jnp
from jax import lax
import jax.experimental.pallas as pl
import jax.experimental.pallas.tpu as pltpu

_NT = (((1,), (1,)), ((), ()))


@jax.jit
def pallas_standalone__mha_block_cached__near_ridge_kernel(x, k_cache, v_cache, wq, wo):
    B, Sq, D = x.shape
    _, H, Sk, Dh = k_cache.shape
    N = B * H
    f32, bf16 = jnp.float32, jnp.bfloat16
    ns, nch = 3, 8
    L = ns - 1
    ck = Sk // nch
    scale = Dh ** -0.5
    items = []
    for o in range(0, 512, 64):
        for t in (0, 1):
            for s in range(4):
                items.append((t, s * 512 + o, 64, s % 2))

    def kern(x_hbm, k_hbm, v_hbm, wq_hbm, wot_hbm, o_hbm, xb, wqb, wob, kb, vb, acc, ob, s_ref, sems, wsem, osem):
        def desc(i, slot, it):
            t, off, nr, p = it
            src = (k_hbm, v_hbm)[t]
            dst = (kb, vb)[t]
            pltpu.make_async_copy(src.at[i, pl.ds(off, nr)], dst.at[slot, pl.ds(off, nr)], sems.at[t, slot]).start(priority=p)

        def wait(t, slot):
            buf = (kb, vb)[t]
            pltpu.make_async_copy(buf.at[slot], buf.at[slot], sems.at[t, slot]).wait()

        cx = pltpu.make_async_copy(x_hbm, xb, wsem.at[0])
        cx.start()
        cq = [pltpu.make_async_copy(wq_hbm.at[:, pl.ds(h * Dh, Dh)], wqb.at[h], wsem.at[1]) for h in range(H)]
        co = [pltpu.make_async_copy(wot_hbm.at[:, pl.ds(h * Dh, Dh)], wob.at[h], wsem.at[2]) for h in range(H)]
        for c in cq:
            c.start()
        for c in co:
            c.start(priority=1)
        for j in range(L):
            for it in items:
                desc(j, j, it)
        cx.wait()
        for c in cq:
            c.wait()
        for c in co:
            c.wait()

        def unit(i, issue):
            b = i // H
            h = lax.rem(i, H)
            slot = lax.rem(i, ns)
            nslot = lax.rem(i + L, ns)
            npts = 2 * nch
            n = len(items)

            def point(j):
                if issue:
                    for it in items[(j * n) // npts:((j + 1) * n) // npts]:
                        desc(i + L, nslot, it)

            wait(0, slot)
            wait(1, slot)
            q = jnp.dot(xb[b], wqb[h], preferred_element_type=f32)
            q = (q * scale).astype(bf16)
            m = None
            for c in range(nch):
                point(c)
                s = lax.dot_general(q, kb[slot, pl.ds(c * ck, ck), :], _NT, preferred_element_type=f32)
                s_ref[:, pl.ds(c * ck, ck)] = s
                for j in range(ck // 128):
                    sj = s[:, j * 128:(j + 1) * 128]
                    m = sj if m is None else jnp.maximum(m, sj)
            m = jnp.max(m, axis=-1, keepdims=True)
            o = None
            l = None
            for c in range(nch):
                point(nch + c)
                p = jnp.exp(s_ref[:, pl.ds(c * ck, ck)] - m)
                for j in range(ck // 128):
                    pj = p[:, j * 128:(j + 1) * 128]
                    l = pj if l is None else l + pj
                oc = jnp.dot(p.astype(bf16), vb[slot, pl.ds(c * ck, ck), :], preferred_element_type=f32)
                o = oc if o is None else o + oc
            l = jnp.sum(l, axis=-1, keepdims=True)
            o = (o * (1.0 / l)).astype(bf16)
            y = lax.dot_general(o, wob[h], _NT, preferred_element_type=f32)
            y = y + jnp.where(h == 0, 0.0, acc[...])
            acc[...] = y
            ob[b] = y.astype(ob.dtype)

        acc[...] = jnp.zeros_like(acc)
        lax.fori_loop(0, N - L, lambda i, _: unit(i, True), None)
        lax.fori_loop(N - L, N, lambda i, _: unit(i, False), None)
        oc = pltpu.make_async_copy(ob, o_hbm, osem.at[0])
        oc.start()
        oc.wait()

    return pl.pallas_call(
        kern,
        in_specs=[pl.BlockSpec(memory_space=pltpu.HBM)] * 5,
        out_specs=pl.BlockSpec(memory_space=pltpu.HBM),
        out_shape=jax.ShapeDtypeStruct((B, Sq, D), x.dtype),
        scratch_shapes=[
            pltpu.VMEM((B, Sq, D), bf16), pltpu.VMEM((H, D, Dh), bf16), pltpu.VMEM((H, D, Dh), bf16),
            pltpu.VMEM((ns, Sk, Dh), bf16), pltpu.VMEM((ns, Sk, Dh), bf16),
            pltpu.VMEM((Sq, D), f32), pltpu.VMEM((B, Sq, D), bf16), pltpu.VMEM((Sq, Sk), f32),
            pltpu.SemaphoreType.DMA((2, ns)), pltpu.SemaphoreType.DMA((3,)), pltpu.SemaphoreType.DMA((1,)),
        ],
        compiler_params=pltpu.CompilerParams(vmem_limit_bytes=100 * 2**20),
    )(x, k_cache.reshape(N, Sk, Dh), v_cache.reshape(N, Sk, Dh), wq, wo.T)
```

```python
import functools

import jax
import jax.numpy as jnp
from jax import lax
import jax.experimental.pallas as pl
import jax.experimental.pallas.tpu as pltpu

_NT = (((1,), (1,)), ((), ()))

_PIECE = 64
_CHUNK = 128
_RING = 4
_QUARTERS = 4

_PIECE_IN_QUARTER = tuple(2 * (j & 1) + ((j >> 1) & 1) + 16 * ((j >> 2) & 1) for j in range(16))
_PIECES_PER_QUARTER = 4

_LEAD = (10, 9)
_LEAD_DROPS = {
    (0, 0): (10, 8, 5, 4, 2),
    (0, 1): (10, 8),
    (1, 0): (10, 8, 5, 4, 3, 2),
    (1, 1): (10, 8),
}


def _mha_kernel(x_hbm, k_hbm, v_hbm, wq_hbm, wot_hbm, out_hbm,
                x_vm, wq_vm, wot_vm, kv_vm, acc_vm, out_vm, s_vm, q_vm, o_vm, l_vm,
                k_sem, v_sem, in_sem, out_sem,
                *, batch, heads, q_len, k_len):
    f32, bf16 = jnp.float32, jnp.bfloat16
    d_model = x_hbm.shape[1]
    d_head = k_hbm.shape[1]
    n_units = batch * heads
    n_chunks = k_len // _CHUNK
    scale = d_head ** -0.5
    kv_hbm, kv_sem = (k_hbm, v_hbm), (k_sem, v_sem)

    def static(i):
        return isinstance(i, int)

    def aligned(start, size, multiple):
        return pl.ds(start if static(start) else pl.multiple_of(start, multiple), size)

    def start_piece(t, row, slot, queue):
        pltpu.make_async_copy(
            kv_hbm[t].at[aligned(row, _PIECE, _PIECE)],
            kv_vm.at[t, aligned(row & (_RING * k_len - 1), _PIECE, _PIECE)],
            kv_sem[t].at[slot],
        ).start(priority=queue)

    def wait_unit(t, slot):
        dst = kv_vm.at[t, aligned(slot * k_len, k_len, _PIECE)]
        pltpu.make_async_copy(dst, dst, kv_sem[t].at[slot]).wait()

    def quarter_target(unit, quarter):
        row = unit * k_len + (_PIECE * _PIECES_PER_QUARTER * quarter - _PIECE)
        if static(quarter):
            first = unit - 1 if quarter == 0 else unit
        else:
            first = jnp.where(quarter == 0, unit - 1, unit)
        return row, first, unit

    def start_issuer(i):
        cache = {}

        def target(t, queue, r):
            drops = _LEAD_DROPS[t, queue]
            key = (_LEAD[t], drops, r)
            if key not in cache:
                if static(i):
                    dropped = sum(i >= n_units - d for d in drops)
                    just_dropped = (n_units - i) in drops
                else:
                    dropped = sum((i >= n_units - d).astype(jnp.int32) for d in drops)
                    just_dropped = dropped > sum((i > n_units - d).astype(jnp.int32) for d in drops)
                g = _QUARTERS * i + (r + _LEAD[t]) - dropped
                row, first, unit = quarter_target(g >> 2, g & 3)
                ok_first, ok = first < n_units, unit < n_units
                if r == 0:
                    if static(i):
                        ok_first, ok = ok_first and not just_dropped, ok and not just_dropped
                    else:
                        keep = jnp.logical_not(just_dropped)
                        ok_first, ok = jnp.logical_and(ok_first, keep), jnp.logical_and(ok, keep)
                cache[key] = (row, first & (_RING - 1), ok_first, unit & (_RING - 1), ok)
            return cache[key]

        def start(j):
            t, queue, piece = (j >> 3) & 1, j & 1, _PIECE_IN_QUARTER[j % 16]
            row, slot_first, ok_first, slot, ok = target(t, queue, j // 16)
            if piece == 0:
                slot, ok = slot_first, ok_first
            go = functools.partial(start_piece, t, row + _PIECE * piece, slot, queue)
            if isinstance(ok, bool):
                if ok:
                    go()
            else:
                pl.when(ok)(go)

        return start

    x_pieces = batch * q_len // 32

    def x_body(j, _):
        for queue in range(2):
            rows = aligned((queue * (x_pieces // 2) + j) * 32, 32, 32)
            pltpu.make_async_copy(x_hbm.at[rows], x_vm.at[rows], in_sem.at[0]).start(priority=queue)

    lax.fori_loop(0, x_pieces // 2, x_body, None)

    w_pieces, w_cols, w_streams = 2 * d_model // 8, heads * d_head // 2, 4

    def w_body(j, _):
        pair = j // 2
        pair = lax.rem(pair, w_streams) * (w_pieces // 2 // w_streams) + pair // w_streams
        piece = pair * 2 + lax.rem(j, 2) + 1
        piece = jnp.where(piece >= w_pieces, piece - w_pieces, piece)
        rows = aligned((piece // 2) * 8, 8, 8)
        cols = aligned(lax.rem(piece, 2) * w_cols, w_cols, 128)
        for queue, (src, dst) in enumerate(((wq_hbm, wq_vm), (wot_hbm, wot_vm))):
            pltpu.make_async_copy(
                src.at[rows, cols], dst.at[rows, cols], in_sem.at[1 + queue]
            ).start(priority=queue)

    lax.fori_loop(0, w_pieces, w_body, None)

    for q in range(-max(_LEAD), 0):
        for j in range(16):
            t, piece = j >> 3, _PIECE_IN_QUARTER[j]
            g = q + _LEAD[t]
            row, first, unit = quarter_target(g >> 2, g & 3)
            row += _PIECE * piece
            if g >= 0 and row >= 0:
                start_piece(t, row, (first if piece == 0 else unit) % _RING, j & 1)

    pltpu.make_async_copy(x_hbm, x_vm, in_sem.at[0]).wait()
    pltpu.make_async_copy(wq_hbm, wq_vm, in_sem.at[1]).wait()
    pltpu.make_async_copy(wot_hbm, wot_vm, in_sem.at[2]).wait()

    def batch_head(u):
        return (u // heads, u % heads) if static(u) else (lax.div(u, heads), lax.rem(u, heads))

    def q_rows(b):
        return aligned(b * q_len, q_len, 16)

    def q_proj(b, h, half):
        cols = aligned(h * d_head + half * 128, 128, 128)
        q = jnp.dot(x_vm[q_rows(b), :], wq_vm[:, cols], preferred_element_type=f32)
        return (q * scale).astype(bf16)

    def out_proj(b, h, o, half):
        lo, n = (0, 256) if half == 0 else (256, d_model - 256)
        w = wot_vm[pl.ds(lo, n), aligned(h * d_head, d_head, 128)]
        y = lax.dot_general(o, w, _NT, preferred_element_type=f32)
        y = y + jnp.where(h == 0, 0.0, acc_vm[:, pl.ds(lo, n)])
        acc_vm[:, pl.ds(lo, n)] = y
        out_vm[q_rows(b), pl.ds(lo, n)] = y.astype(out_vm.dtype)

    def normalized(o, l):
        return (o * (1.0 / jnp.sum(l, axis=-1, keepdims=True))).astype(bf16)

    def write_rows(lo, n, queue):
        rows = pl.ds(lo, n)
        pltpu.make_async_copy(out_vm.at[rows], out_hbm.at[rows], out_sem.at[0]).start(priority=queue)

    def step(i, last):
        slot = i & (_RING - 1)
        b_prev, h_prev = batch_head(i - 1 if static(i) else jnp.maximum(i - 1, 0))
        if not last:
            b_next, h_next = batch_head(i + 1)
        q = q_vm[...]
        start = start_issuer(i)

        def kv_chunk(t, c):
            return kv_vm[t, aligned(slot * k_len + c * _CHUNK, _CHUNK, _PIECE), :]

        wait_unit(0, slot)
        m = None
        for c in range(n_chunks):
            s = lax.dot_general(q, kv_chunk(0, c), _NT, preferred_element_type=f32)
            s_vm[:, pl.ds(c * _CHUNK, _CHUNK)] = s
            m = s if m is None else jnp.maximum(m, s)
            start(2 * c)
            start(2 * c + 1)
            if c == 0:
                o_prev = normalized(o_vm[...], l_vm[...])
            if c == (11 if last else 7):
                out_proj(b_prev, h_prev, o_prev, 0)
                if last:
                    done = (batch - 1) * q_len
                    half = done // 32 * 16
                    write_rows(0, half, 0)
                    write_rows(half, done - half, 1)
        m = jnp.max(m, axis=-1, keepdims=True)
        out_proj(b_prev, h_prev, o_prev, 1)
        if not last:
            q_next = [q_proj(b_next, h_next, 0)]

        wait_unit(1, slot)
        o = l = None
        for c in range(n_chunks):
            p = jnp.exp(s_vm[:, pl.ds(c * _CHUNK, _CHUNK)] - m)
            l = p if l is None else l + p
            pv = jnp.dot(p.astype(bf16), kv_chunk(1, c), preferred_element_type=f32)
            o = pv if o is None else o + pv
            start(2 * (n_chunks + c))
            start(2 * (n_chunks + c) + 1)
            if c == 7 and not last:
                q_next.append(q_proj(b_next, h_next, 1))

        if last:
            o = normalized(o, l)
            for half in range(2):
                out_proj(batch - 1, heads - 1, o, half)
        else:
            o_vm[...] = o
            l_vm[...] = l
            for half in range(2):
                q_vm[:, pl.ds(half * 128, 128)] = q_next[half]

    acc_vm[...] = jnp.zeros_like(acc_vm)
    o_vm[...] = jnp.zeros_like(o_vm)
    l_vm[...] = jnp.ones_like(l_vm)
    for half in range(2):
        q_vm[:, pl.ds(half * 128, 128)] = q_proj(0, 0, half)

    lax.fori_loop(0, n_units - 1, lambda i, _: step(i, False), None)
    step(n_units - 1, True)

    write_rows((batch - 1) * q_len, q_len, 0)
    pltpu.make_async_copy(out_vm, out_hbm, out_sem.at[0]).wait()


@jax.jit
def pallas_standalone__mha_block_cached__near_ridge_kernel(
    x: jax.Array,
    k_cache: jax.Array,
    v_cache: jax.Array,
    wq: jax.Array,
    wo: jax.Array,
):
    batch, q_len, d_model = x.shape
    _, heads, k_len, d_head = k_cache.shape
    assert (k_len, d_head) == (2048, 256) and batch * heads > 10
    assert q_len % 16 == 0 and (batch * q_len) % 64 == 0
    assert d_model % 32 == 0 and d_model > 256

    f32, bf16 = jnp.float32, jnp.bfloat16
    rows = batch * q_len
    out = pl.pallas_call(
        functools.partial(_mha_kernel, batch=batch, heads=heads, q_len=q_len, k_len=k_len),
        in_specs=[pl.BlockSpec(memory_space=pltpu.HBM)] * 5,
        out_specs=pl.BlockSpec(memory_space=pltpu.HBM),
        out_shape=jax.ShapeDtypeStruct((rows, d_model), x.dtype),
        scratch_shapes=[
            pltpu.VMEM((rows, d_model), bf16),
            pltpu.VMEM((d_model, heads * d_head), bf16),
            pltpu.VMEM((d_model, heads * d_head), bf16),
            pltpu.VMEM((2, _RING * k_len, d_head), bf16),
            pltpu.VMEM((q_len, d_model), f32),
            pltpu.VMEM((rows, d_model), x.dtype),
            pltpu.VMEM((q_len, k_len), f32),
            pltpu.VMEM((q_len, d_head), bf16),
            pltpu.VMEM((q_len, d_head), f32),
            pltpu.VMEM((q_len, _CHUNK), f32),
            pltpu.SemaphoreType.DMA((_RING,)),
            pltpu.SemaphoreType.DMA((_RING,)),
            pltpu.SemaphoreType.DMA((3,)),
            pltpu.SemaphoreType.DMA((1,)),
        ],
        compiler_params=pltpu.CompilerParams(
            vmem_limit_bytes=64 * 2**20, disable_bounds_checks=True
        ),
    )(
        x.reshape(rows, d_model),
        k_cache.reshape(batch * heads * k_len, d_head),
        v_cache.reshape(batch * heads * k_len, d_head),
        wq,
        wo.T,
    )
    return out.reshape(batch, q_len, d_model)
```

```python
import functools

import jax
import jax.numpy as jnp
from jax import lax
import jax.experimental.pallas as pl
import jax.experimental.pallas.tpu as pltpu

_NT = (((1,), (1,)), ((), ()))

_PIECE = 64
_CHUNK = 128
_RING = 4
_QUARTERS = 4

_PIECE_IN_QUARTER = tuple(2 * (j & 1) + ((j >> 1) & 1) + 16 * ((j >> 2) & 1) for j in range(16))
_PIECES_PER_QUARTER = 4

_LEAD = (9, 7)
_LEAD_DROPS = {
    (0, 0): (8, 5, 4, 2),
    (0, 1): (8,),
    (1, 0): (5, 4, 3, 2),
    (1, 1): (8, 2),
}


def _mha_kernel(x_hbm, k_hbm, v_hbm, wq_hbm, wot_hbm, out_hbm,
                x_vm, wq_vm, wot_vm, kv_vm, acc_vm, out_vm, s_vm, q_vm, o_vm, l_vm,
                k_sem, v_sem, in_sem, out_sem,
                *, batch, heads, q_len, k_len):
    f32, bf16 = jnp.float32, jnp.bfloat16
    d_model = x_hbm.shape[1]
    d_head = k_hbm.shape[1]
    n_units = batch * heads
    n_chunks = k_len // _CHUNK
    scale = d_head ** -0.5
    kv_hbm, kv_sem = (k_hbm, v_hbm), (k_sem, v_sem)

    def static(i):
        return isinstance(i, int)

    def aligned(start, size, multiple):
        return pl.ds(start if static(start) else pl.multiple_of(start, multiple), size)

    def start_piece(t, row, slot, queue):
        pltpu.make_async_copy(
            kv_hbm[t].at[aligned(row, _PIECE, _PIECE)],
            kv_vm.at[t, aligned(row & (_RING * k_len - 1), _PIECE, _PIECE)],
            kv_sem[t].at[slot],
        ).start(priority=queue)

    def wait_unit(t, slot):
        dst = kv_vm.at[t, aligned(slot * k_len, k_len, _PIECE)]
        pltpu.make_async_copy(dst, dst, kv_sem[t].at[slot]).wait()

    def quarter_target(unit, quarter):
        row = unit * k_len + (_PIECE * _PIECES_PER_QUARTER * quarter - _PIECE)
        if static(quarter):
            first = unit - 1 if quarter == 0 else unit
        else:
            first = jnp.where(quarter == 0, unit - 1, unit)
        return row, first, unit

    def start_issuer(i):
        cache = {}

        def target(t, queue, r):
            drops = _LEAD_DROPS[t, queue]
            key = (_LEAD[t], drops, r)
            if key not in cache:
                if static(i):
                    dropped = sum(i >= n_units - d for d in drops)
                    just_dropped = (n_units - i) in drops
                else:
                    dropped = sum((i >= n_units - d).astype(jnp.int32) for d in drops)
                    just_dropped = dropped > sum((i > n_units - d).astype(jnp.int32) for d in drops)
                g = _QUARTERS * i + (r + _LEAD[t]) - dropped
                row, first, unit = quarter_target(g >> 2, g & 3)
                ok_first, ok = first < n_units, unit < n_units
                if r == 0:
                    if static(i):
                        ok_first, ok = ok_first and not just_dropped, ok and not just_dropped
                    else:
                        keep = jnp.logical_not(just_dropped)
                        ok_first, ok = jnp.logical_and(ok_first, keep), jnp.logical_and(ok, keep)
                cache[key] = (row, first & (_RING - 1), ok_first, unit & (_RING - 1), ok)
            return cache[key]

        def start(j):
            t, queue, piece = (j >> 3) & 1, j & 1, _PIECE_IN_QUARTER[j % 16]
            row, slot_first, ok_first, slot, ok = target(t, queue, j // 16)
            if piece == 0:
                slot, ok = slot_first, ok_first
            go = functools.partial(start_piece, t, row + _PIECE * piece, slot, queue)
            if isinstance(ok, bool):
                if ok:
                    go()
            else:
                pl.when(ok)(go)

        return start

    def x_body(j, _):
        rows = aligned(j * 32, 32, 32)
        pltpu.make_async_copy(x_hbm.at[rows], x_vm.at[rows], in_sem.at[0]).start(priority=1)

    lax.fori_loop(0, batch * q_len // 32, x_body, None)

    w_pieces, w_cols, w_streams = 2 * d_model // 8, heads * d_head // 2, 4

    def w_body(j, _):
        pair = j // 2
        pair = lax.rem(pair, w_streams) * (w_pieces // 2 // w_streams) + pair // w_streams
        piece = pair * 2 + lax.rem(j, 2) + 1
        piece = jnp.where(piece >= w_pieces, piece - w_pieces, piece)
        rows = aligned((piece // 2) * 8, 8, 8)
        cols = aligned(lax.rem(piece, 2) * w_cols, w_cols, 128)
        for queue, (src, dst) in enumerate(((wq_hbm, wq_vm), (wot_hbm, wot_vm))):
            pltpu.make_async_copy(
                src.at[rows, cols], dst.at[rows, cols], in_sem.at[1 + queue]
            ).start(priority=queue)

    lax.fori_loop(0, w_pieces, w_body, None)

    for q in range(-max(_LEAD), 0):
        for j in range(16):
            t, piece = j >> 3, _PIECE_IN_QUARTER[j]
            g = q + _LEAD[t]
            row, first, unit = quarter_target(g >> 2, g & 3)
            row += _PIECE * piece
            if g >= 0 and row >= 0:
                start_piece(t, row, (first if piece == 0 else unit) % _RING, j & 1)

    pltpu.make_async_copy(x_hbm, x_vm, in_sem.at[0]).wait()
    pltpu.make_async_copy(wq_hbm, wq_vm, in_sem.at[1]).wait()
    pltpu.make_async_copy(wot_hbm, wot_vm, in_sem.at[2]).wait()

    def batch_head(u):
        return (u // heads, u % heads) if static(u) else (lax.div(u, heads), lax.rem(u, heads))

    def q_rows(b):
        return aligned(b * q_len, q_len, 16)

    def q_proj(b, h):
        w = wq_vm[:, aligned(h * d_head, d_head, 128)]
        q = jnp.dot(x_vm[q_rows(b), :], w, preferred_element_type=f32)
        return (q * scale).astype(bf16)

    def out_proj(b, h, o, half):
        lo, n = (0, 256) if half == 0 else (256, d_model - 256)
        w = wot_vm[pl.ds(lo, n), aligned(h * d_head, d_head, 128)]
        y = lax.dot_general(o, w, _NT, preferred_element_type=f32)
        y = y + jnp.where(h == 0, 0.0, acc_vm[:, pl.ds(lo, n)])
        acc_vm[:, pl.ds(lo, n)] = y
        out_vm[q_rows(b), pl.ds(lo, n)] = y.astype(out_vm.dtype)

    def normalized(o, l):
        return (o * (1.0 / jnp.sum(l, axis=-1, keepdims=True))).astype(bf16)

    def write_rows(lo, n, queue):
        rows = pl.ds(lo, n)
        pltpu.make_async_copy(out_vm.at[rows], out_hbm.at[rows], out_sem.at[0]).start(priority=queue)

    def step(i, last):
        slot = i & (_RING - 1)
        b_prev, h_prev = batch_head(i - 1 if static(i) else jnp.maximum(i - 1, 0))
        if not last:
            b_next, h_next = batch_head(i + 1)
        q = q_vm[...]
        start = start_issuer(i)

        def kv_chunk(t, c):
            return kv_vm[t, aligned(slot * k_len + c * _CHUNK, _CHUNK, _PIECE), :]

        wait_unit(0, slot)
        m = None
        for c in range(n_chunks):
            s = lax.dot_general(q, kv_chunk(0, c), _NT, preferred_element_type=f32)
            s_vm[:, pl.ds(c * _CHUNK, _CHUNK)] = s
            m = s if m is None else jnp.maximum(m, s)
            start(2 * c)
            start(2 * c + 1)
            if c == 0:
                o_prev = normalized(o_vm[...], l_vm[...])
            if c == (11 if last else 3):
                out_proj(b_prev, h_prev, o_prev, 0)
                if last:
                    done = (batch - 1) * q_len
                    half = done // 32 * 16
                    write_rows(0, half, 0)
                    write_rows(half, done - half, 1)
            if c == (n_chunks - 1 if last else 9):
                out_proj(b_prev, h_prev, o_prev, 1)
        m = jnp.max(m, axis=-1, keepdims=True)
        if not last:
            q_next = q_proj(b_next, h_next)

        wait_unit(1, slot)
        o = l = None
        for c in range(n_chunks):
            p = jnp.exp(s_vm[:, pl.ds(c * _CHUNK, _CHUNK)] - m)
            l = p if l is None else l + p
            pv = jnp.dot(p.astype(bf16), kv_chunk(1, c), preferred_element_type=f32)
            o = pv if o is None else o + pv
            start(2 * (n_chunks + c))
            start(2 * (n_chunks + c) + 1)

        if last:
            o = normalized(o, l)
            for half in range(2):
                out_proj(batch - 1, heads - 1, o, half)
        else:
            o_vm[...] = o
            l_vm[...] = l
            q_vm[...] = q_next

    acc_vm[...] = jnp.zeros_like(acc_vm)
    o_vm[...] = jnp.zeros_like(o_vm)
    l_vm[...] = jnp.ones_like(l_vm)
    q_vm[...] = q_proj(0, 0)

    lax.fori_loop(0, n_units - 1, lambda i, _: step(i, False), None)
    step(n_units - 1, True)

    write_rows((batch - 1) * q_len, q_len, 0)
    pltpu.make_async_copy(out_vm, out_hbm, out_sem.at[0]).wait()


@jax.jit
def pallas_standalone__mha_block_cached__near_ridge_kernel(
    x: jax.Array,
    k_cache: jax.Array,
    v_cache: jax.Array,
    wq: jax.Array,
    wo: jax.Array,
):
    batch, q_len, d_model = x.shape
    _, heads, k_len, d_head = k_cache.shape
    assert (k_len, d_head) == (2048, 256) and batch > 1 and batch * heads > 8
    assert q_len % 16 == 0 and (batch * q_len) % 32 == 0
    assert d_model % 32 == 0 and d_model > 256

    f32, bf16 = jnp.float32, jnp.bfloat16
    rows = batch * q_len
    out = pl.pallas_call(
        functools.partial(_mha_kernel, batch=batch, heads=heads, q_len=q_len, k_len=k_len),
        in_specs=[pl.BlockSpec(memory_space=pltpu.HBM)] * 5,
        out_specs=pl.BlockSpec(memory_space=pltpu.HBM),
        out_shape=jax.ShapeDtypeStruct((rows, d_model), x.dtype),
        scratch_shapes=[
            pltpu.VMEM((rows, d_model), bf16),
            pltpu.VMEM((d_model, heads * d_head), bf16),
            pltpu.VMEM((d_model, heads * d_head), bf16),
            pltpu.VMEM((2, _RING * k_len, d_head), bf16),
            pltpu.VMEM((q_len, d_model), f32),
            pltpu.VMEM((rows, d_model), x.dtype),
            pltpu.VMEM((q_len, k_len), f32),
            pltpu.VMEM((q_len, d_head), bf16),
            pltpu.VMEM((q_len, d_head), f32),
            pltpu.VMEM((q_len, _CHUNK), f32),
            pltpu.SemaphoreType.DMA((_RING,)),
            pltpu.SemaphoreType.DMA((_RING,)),
            pltpu.SemaphoreType.DMA((3,)),
            pltpu.SemaphoreType.DMA((1,)),
        ],
        compiler_params=pltpu.CompilerParams(
            vmem_limit_bytes=64 * 2**20, disable_bounds_checks=True
        ),
    )(
        x.reshape(rows, d_model),
        k_cache.reshape(batch * heads * k_len, d_head),
        v_cache.reshape(batch * heads * k_len, d_head),
        wq,
        wo.T,
    )
    return out.reshape(batch, q_len, d_model)
```
